```python
import os as _os
_os.environ.setdefault("JAX_PLATFORMS", "cpu")
import jax
import jax.numpy as jnp

def _softmax(x, axis=-1):
    return jax.nn.softmax(x, axis=axis)
def _gelu(x):
    return jax.nn.gelu(x, approximate=True)
def _silu(x):
    return jax.nn.silu(x)
def _sigmoid(x):
    return jax.nn.sigmoid(x)
def _layernorm(x, axis=-1, eps=1e-5):
    m = jnp.mean(x, axis=axis, keepdims=True)
    v = jnp.var(x, axis=axis, keepdims=True)
    return (x - m) / jnp.sqrt(v + eps)
def _scatter_add(tgt, idx, src, axis=0):
    return tgt.at[idx].add(src)
def _segment_sum(src, seg, n):
    return jax.ops.segment_sum(src, seg, n)
class _Rng:
    def __init__(self, key):
        self._k = key
    def _next(self):
        self._k, sub = jax.random.split(self._k)
        return sub
    def normal(self, shape):
        return jax.random.normal(self._next(), shape, dtype=jnp.bfloat16)
    def randint(self, lo, hi, shape):
        return jax.random.randint(self._next(), shape, lo, hi, dtype=jnp.int32)
    def uniform(self, shape, lo=0.0, hi=1.0):
        return jax.random.uniform(self._next(), shape, jnp.bfloat16, lo, hi)
    def permutation(self, n):
        return jax.random.permutation(self._next(), n)


kernel_name = 'standalone__glu_gated_bilinear__prompt'

def setup_inputs():
    _rng = _Rng(jax.random.key(int.from_bytes(__import__("os").urandom(4), "little")))
    _w = (lambda a: (lambda t: t.astype(jnp.bfloat16) if jnp.issubdtype(t.dtype, jnp.floating) else t)(jnp.asarray(a)))
    B, S, D, F = 1, 2048, 640, 1728
    return {
        "x": _w((lambda *s: _rng.normal(s) * 0.05)(B, S, D)),
        "w_gate": _w((lambda *s: _rng.normal(s) * 0.05)(D, F) * (D ** -0.5)),
        "w_up": _w((lambda *s: _rng.normal(s) * 0.05)(D, F) * (D ** -0.5)),
        "w_down": _w((lambda *s: _rng.normal(s) * 0.05)(F, D) * (F ** -0.5)),
    }

def reference(x, w_gate, w_up, w_down):
    g = jnp.einsum("bsd,df->bsf", x, w_gate)
    u = jnp.einsum("bsd,df->bsf", x, w_up)
    h = g * u
    return jnp.einsum("bsf,fd->bsd", h, w_down)
```

```python
import functools, itertools
import numpy as np
import jax, jax.numpy as jnp
from jax import lax
from jax.experimental import pallas as pl
from jax.experimental.pallas import tpu as pltpu

NT = (((1,), (1,)), ((), ()))
f32, bf16 = jnp.float32, jnp.bfloat16
S, D, F = 2048, 640, 1728
T = 128
G = 5

def dnt(a, b): return lax.dot_general(a, b, NT, preferred_element_type=f32)
def dnn(a, b): return jnp.dot(a, b, preferred_element_type=f32)
PAIRS = list(itertools.combinations(range(G), 2))

def comb(a, b, sign, n):
    op = (lambda p, q: p + q) if sign > 0 else (lambda p, q: p - q)
    ra, rb = min(a.shape[0], n), min(b.shape[0], n)
    c = min(ra, rb)
    head = op(a[:c], b[:c])
    if c == n: return head
    tail = a[c:n] if ra > rb else (b[c:n] if sign > 0 else -b[c:n])
    return jnp.concatenate([head, tail], 0)

def make(mA=(208,208,208,208,192), mB=(192,208,208,208,208), npi=3, stages=(2, 5, 10), ostages=(8,), g1style="acc",
         phases="012", flags=None, nobc=False, nosc=False, g2mode="sep"):
    NP = 6
    sizes = list(mA) + list(mB)
    offs = [int(v) for v in np.cumsum([0] + sizes)]
    assert offs[-1] == S
    pos = {}; n = 0
    def put(key, rows):
        nonlocal n
        pos[key] = (n, rows); n += rows
    for k in range(G):
        put(('3', k), mA[k]); put(('4', k), mB[k]); put(('5', k), mA[k]); put(('2', k), mB[k])
        put(('A', k, k), mA[k]); put(('B', k, k), mB[k])
    for (k, l) in PAIRS:
        put(('1', k, l), max(mA[k], mB[l])); put(('1', l, k), max(mA[l], mB[k]))
        put(('B', l, k), mB[l]); put(('B', k, l), mB[k])
        put(('A', k, l), mA[k]); put(('A', l, k), mA[l])
    NL = n
    def span(a, b=None):
        s, r = pos[a]
        if b is not None:
            assert pos[b][0] == s + r
            r += pos[b][1]
        return pl.ds(s, r)
    gkey = lambda g, k: ('A', g, k) if g < G else ('B', g - G, k)
    rows = lambda g: pl.ds(offs[g], sizes[g])

    def kern(x_hbm, wg_hbm, wu_hbm, wd_hbm, o_hbm, lx, wg_v, wu_v, wt_v, wd_v, h_v, o_v, sem):
        cp = pltpu.make_async_copy
        col = lambda k: pl.ds(k * T, T)
        grp = []
        first = [cp(wg_hbm.at[pl.ds(1536, T)], wt_v.at[pl.ds(0, T)], sem.at[0]),
                 cp(wu_hbm.at[pl.ds(1536, T)], wt_v.at[pl.ds(T, T)], sem.at[0]),
                 cp(wg_hbm.at[pl.ds(1664, 64)], wt_v.at[pl.ds(2 * T, 64)], sem.at[0]),
                 cp(wu_hbm.at[pl.ds(1664, 64)], wt_v.at[pl.ds(2 * T + 64, 64)], sem.at[0])]
        g0 = 0
        for si, g1 in enumerate(stages):
            c = first if si == 0 else []
            for g in range(g0, g1):
                c += [cp(x_hbm.at[rows(g), col(k)], lx.at[span(gkey(g, k))], sem.at[si]) for k in range(G)]
            grp.append(c); g0 = g1
        ns = len(stages)
        nit = NP // npi
        def wcopies(it):
            r = pl.ds(it * npi * 2 * T, npi * 2 * T)
            return [cp(wg_hbm.at[r], wg_v.at[r], sem.at[ns + it]), cp(wu_hbm.at[r], wu_v.at[r], sem.at[ns + it])]
        wdc = [cp(wd_hbm.at[:, col(k)], wd_v.at[k, pl.ds(0, F)], sem.at[ns + nit]) for k in range(G)]
        osem = sem.at[ns + nit + 1]
        for c in sum(grp, []) + sum((wcopies(i) for i in range(nit)), []) + wdc: c.start()
        for k in range(G):
            wd_v[k, pl.ds(F, 64), :] = jnp.zeros((64, T), bf16)

        xf = lambda key: lx[span(key), :].astype(f32)
        def rowsum(name, kind, k):
            v = xf((kind, k, k))
            for l in range(G):
                if l != k: v = v - xf((kind, k, l))
            lx[span((name, k)), :] = v.astype(bf16)
        def colsum(name, kind, other, k):
            v = xf((kind, k, k))
            for l in range(G):
                if l != k: v = comb(v, xf((other, l, k)), 1, v.shape[0])
            lx[span((name, k)), :] = v.astype(bf16)
        g0 = 0
        for si, g1 in enumerate(stages):
            for c in grp[si]: c.wait()
            if '0' not in phases: continue
            for g in range(g0, g1):
                acc = [None] * 3
                for k in range(G):
                    xt = lx[span(gkey(g, k)), :]
                    for t in range(3):
                        d = dnt(xt, wt_v[pl.ds(t * T, T), col(k)])
                        acc[t] = d if acc[t] is None else acc[t] + d
                ht = acc[2] * pltpu.roll(acc[2], 64, 1)
                lane = lax.broadcasted_iota(jnp.int32, ht.shape, 1)
                h_v[0, NP, rows(g), :] = acc[0] * acc[1]
                h_v[1, NP, rows(g), :] = jnp.where(lane < 64, ht, 0.0)
                if g < G: rowsum('5', 'A', g)
                else:
                    l = g - G
                    rowsum('2', 'B', l)
                    colsum('4', 'B', 'A', l)
                    for k in range(G):
                        if k != l:
                            lx[span(('1', k, l)), :] = comb(xf(('A', k, l)), xf(('B', l, k)), 1, pos['1', k, l][1]).astype(bf16)
            g0 = g1
        if '0' in phases:
            for k in range(G): colsum('3', 'A', 'B', k)

        def g1_body(it, _):
            for c in [pltpu.make_async_copy(w.at[pl.ds(0, npi * 2 * T)], v.at[pl.ds(0, npi * 2 * T)], sem.at[ns + it])
                      for w, v in ((wg_hbm, wg_v), (wu_hbm, wu_v))]:
                c.wait()
            for jj in range(npi):
                j = it * npi + jj
                r = [pl.ds(pl.multiple_of(j * 2 * T + hf * T, T), T) for hf in range(2)]
                W = (wg_v, wu_v)
                b = lambda w, hf, k: w[r[hf], col(k)]
                bf_ = lambda w, hf, k: b(w, hf, k).astype(f32)
                def prod(lhs_span, rhs):
                    lhs = lx[lhs_span, :]
                    return [dnt(lhs, rhs(w)) for w in W]
                a1, a2, c1, c2 = [[None] * G for _ in range(4)]
                def upd(lst, i, v, sign, nrows):
                    lst[i] = v if lst[i] is None else [comb(p, q, sign, nrows) for p, q in zip(lst[i], v)]
                def diag(k):
                    m5 = prod(span(('5', k)), lambda w: b(w, 1, k))
                    m2 = prod(span(('2', k)), lambda w: b(w, 0, k))
                    m34 = prod(span(('3', k), ('4', k)), lambda w: (bf_(w, 0, k) - bf_(w, 1, k)).astype(bf16))
                    upd(a1, k, [p[:mA[k]] + q for p, q in zip(m34, m5)], 1, mA[k]); upd(a2, k, m5, 1, mA[k])
                    upd(c2, k, [q - p[mA[k]:] for p, q in zip(m34, m2)], 1, mB[k]); upd(c1, k, m2, 1, mB[k])
                def finish(k):
                    h_v[0, j, rows(k), :] = a1[k][0] * a1[k][1]
                    h_v[1, j, rows(k), :] = a2[k][0] * a2[k][1]
                    h_v[0, j, rows(G + k), :] = c1[k][0] * c1[k][1]
                    h_v[1, j, rows(G + k), :] = c2[k][0] * c2[k][1]
                done = set()
                for (k, l) in PAIRS:
                    for q in (k, l):
                        if q not in done: diag(q); done.add(q)
                    m6 = prod(span(('B', l, k), ('B', k, l)), lambda w: (bf_(w, 0, k) + bf_(w, 0, l)).astype(bf16))
                    m7 = prod(span(('A', k, l), ('A', l, k)), lambda w: (bf_(w, 1, k) + bf_(w, 1, l)).astype(bf16))
                    for (p, q, s6, s7) in ((k, l, slice(0, mB[l]), slice(0, mA[k])), (l, k, slice(mB[l], None), slice(mA[k], None))):
                        m1 = prod(span(('1', p, q)), lambda w: (bf_(w, 0, q) + bf_(w, 1, p)).astype(bf16))
                        upd(a1, p, [comb(u, v[s6], -1, mA[p]) for u, v in zip(m1, m6)], 1, mA[p])
                        upd(c1, q, [v[s6] for v in m6], 1, mB[q])
                        upd(c2, q, [comb(u, v[s7], -1, mB[q]) for u, v in zip(m1, m7)], 1, mB[q])
                        upd(a2, p, [v[s7] for v in m7], 1, mA[p])
                    if l == G - 1: finish(k)
                finish(G - 1)
            return _
        if '1' in phases:
            if nit == 1: g1_body(0, None)
            else: lax.fori_loop(0, nit, g1_body, None)
        else:
            for i in range(nit):
                for c in wcopies(i): c.wait()

        for c in wdc: c.wait()
        ocp = []
        if '2' in phases:
            def prod(lhs, rhs):
                if g2mode == "cat":
                    return dnn(jnp.concatenate([lhs(j) for j in range(NP + 1)], 1).astype(bf16),
                               jnp.concatenate([rhs(j) for j in range(NP + 1)], 0).astype(bf16))
                out = None
                for j in range(NP + 1):
                    d = dnn(lhs(j).astype(bf16), rhs(j).astype(bf16))
                    out = d if out is None else out + d
                return out
            hb = lambda hf, g: (lambda j: h_v[hf, j, rows(g), :])
            wb = lambda hf, k: (lambda j: wd_v[k, pl.ds((2 * j + hf) * T, T), :])
            lin = lambda f, g, s, n: (lambda j: comb(f(j), g(j), s, n))
            wlin = lambda f, g, s: (lambda j: comb(f(j).astype(f32), g(j).astype(f32), s, T))
            cat = lambda f, g: (lambda j: jnp.concatenate([f(j), g(j)], 0))
            ready = []
            def emit(g, k, v):
                o_v[k, rows(g), :] = v.astype(bf16)
                ready.append((g, k))
            def flush():
                ready.sort(key=lambda t: (t[1], t[0]))
                runs = []
                for g, k in ready:
                    if runs and runs[-1][0] == k and runs[-1][2] == g: runs[-1][2] = g + 1
                    else: runs.append([k, g, g + 1])
                for k, ga, gb in runs:
                    r = pl.ds(offs[ga], offs[gb] - offs[ga])
                    c = cp(o_v.at[k, r], o_hbm.at[r, col(k)], osem); c.start(); ocp.append(c)
                ready.clear()
            M2, M3, M4, M5 = {}, {}, {}, {}
            def diag2(k):
                M5[k] = prod(lin(hb(0, k), hb(1, k), 1, mA[k]), wb(1, k))
                M2[k] = prod(lin(hb(0, G + k), hb(1, G + k), 1, mB[k]), wb(0, k))
                m34 = prod(cat(hb(0, k), hb(1, G + k)), wlin(wb(0, k), wb(1, k), -1))
                M3[k], M4[k] = m34[:mA[k]], m34[mA[k]:]
                emit(k, k, M3[k] + M5[k]); emit(G + k, k, M2[k] - M4[k])
            for pi, (k, l) in enumerate(PAIRS):
                for q in (k, l):
                    if q not in M2: diag2(q)
                m6 = prod(cat(lin(hb(0, G + l), hb(0, k), -1, mB[l]), lin(hb(0, G + k), hb(0, l), -1, mB[k])), wlin(wb(0, k), wb(0, l), 1))
                m7 = prod(cat(lin(hb(1, k), hb(1, G + l), -1, mA[k]), lin(hb(1, l), hb(1, G + k), -1, mA[l])), wlin(wb(1, k), wb(1, l), 1))
                for (p, q, s6, s7) in ((k, l, slice(0, mB[l]), slice(0, mA[k])), (l, k, slice(mB[l], None), slice(mA[k], None))):
                    m1 = prod(lin(hb(0, p), hb(1, G + q), 1, max(mA[p], mB[q])), wlin(wb(0, q), wb(1, p), 1))
                    emit(p, q, comb(m1, M4[q], -1, mA[p]) + (m7[s7] - M5[p]))
                    emit(G + q, p, comb(m1, M3[p], 1, mB[q]) + (m6[s6] - M2[q]))
                if pi + 1 in ostages: flush()
            flush()
        else:
            o_v[0, 0:16, :] = h_v[0, 0, 0:16, :].astype(bf16)
            c = cp(o_v.at[0], o_hbm.at[:, col(0)], osem); c.start(); ocp.append(c)
        for c in ocp: c.wait()

    def fn(x, wg, wu, wd):
        B = x.shape[0]
        hbm = pl.BlockSpec(memory_space=pltpu.HBM)
        out = pl.pallas_call(
            kern, in_specs=[hbm] * 4, out_specs=hbm,
            out_shape=jax.ShapeDtypeStruct((S, D), bf16),
            scratch_shapes=[
                pltpu.VMEM((NL, T), bf16), pltpu.VMEM((1536, D), bf16), pltpu.VMEM((1536, D), bf16),
                pltpu.VMEM((3 * T, D), bf16), pltpu.VMEM((G, F + 64, T), bf16),
                pltpu.VMEM((2, NP + 1, S, T), f32), pltpu.VMEM((G, S, T), bf16),
                pltpu.SemaphoreType.DMA((len(stages) + NP // npi + 2,)),
            ],
            compiler_params=pltpu.CompilerParams(vmem_limit_bytes=110 << 20, flags=flags,
                                                 disable_bounds_checks=nobc, disable_semaphore_checks=nosc),
        )(x.reshape(S, D), wg.T, wu.T, wd)
        return out.reshape(B, S, D)
    return fn


_fn = make(npi=3)

@jax.jit
def pallas_standalone__glu_gated_bilinear__prompt_kernel(x, w_gate, w_up, w_down):
    return _fn(x, w_gate, w_up, w_down)
```

```python
import functools
import itertools

import jax
import jax.numpy as jnp
from jax import lax
import jax.experimental.pallas as pl
import jax.experimental.pallas.tpu as pltpu

S, D, F = 2048, 640, 1728
T = 128
HT = T // 2
G = D // T

SIZES = (208, 208, 208, 208, 192, 192, 208, 208, 208, 208)
OFFSETS = (0, 208, 416, 624, 832, 1856, 1024, 1232, 1440, 1648)
MA, MB = SIZES[:G], SIZES[G:]
MAX_ROWS = max(SIZES)
PAIRS = tuple(itertools.combinations(range(G), 2))

ARRIVALS = (("w0", 0), ("w2",), (1,), (2,), (3,), (4,), (5,), ("w1",),
            (6,), (7,), (8,), (9, "wd"))

F32, BF16 = jnp.float32, jnp.bfloat16


def _others(k):
    return [l for l in range(G) if l != k]


def _longest_first(half):
    return sorted(range(G), key=lambda j: -SIZES[G * half + j])


def _operand_layout():
    pos, used = {}, {"tile": 0, "sum": 0}

    def put(key, rows):
        kind = "tile" if key[0] in "AB" else "sum"
        pos[key] = (used[kind], rows)
        used[kind] += rows

    for k in range(G):
        put(("3", k), MA[k])
        put(("4", k), MB[k])
        put(("5", k), MA[k])
        put(("2", k), MB[k])
        put(("A", k, k), MA[k])
        put(("B", k, k), MB[k])
    for k, l in PAIRS:
        put(("1", k, l), max(MA[k], MB[l]))
        put(("1", l, k), max(MA[l], MB[k]))
        put(("B", l, k), MB[l])
        put(("B", k, l), MB[k])
        put(("A", k, l), MA[k])
        put(("A", l, k), MA[l])
    return pos, used


def _startup_plan():
    plan, done, have = [], set(), set()
    plain_after = {2 * G - 1: 2}
    for items in ARRIVALS:
        have.update(items)
        tasks = []
        has_a = lambda k: k in have
        has_b = lambda k: G + k in have
        w1, w2 = "w1" in have, "w2" in have

        def add(task, ready):
            if ready and task not in done:
                done.add(task)
                tasks.append(task)

        def add_plain(position):
            for g in range(2 * G):
                if plain_after.get(g, 0) == position:
                    add(("plain", g), g in have)

        def hidden_done(q):
            need = [("plain", q), ("plain", G + q)] + [(m, q) for m in "2345"]
            for l in _others(q):
                need += [(m, p, r) for m in "167" for p, r in ((q, l), (l, q))]
            return all(t in done for t in need)

        add_plain(0)
        for k in range(G):
            for l in range(k + 1, G):
                for p, q in ((k, l), (l, k)):
                    add(("7", p, q), w2 and has_a(p))
                for p, q in ((k, l), (l, k)):
                    add(("6", p, q), w1 and has_b(q))
                for p, q in ((k, l), (l, k)):
                    add(("1", p, q), w1 and w2 and has_a(p) and has_b(q))
            add(("5", k), w2 and has_a(k))
            add(("2", k), w1 and has_b(k))
            add(("4", k), w1 and w2 and has_b(k) and all(map(has_a, _others(k))))
            add(("3", k), w1 and w2 and has_a(k) and all(map(has_b, _others(k))))
            add_plain(k + 1)
            if "wd" in have:
                for q in range(k if k < G - 1 else G):
                    add(("down_diag", q), hidden_done(q))
                    for l in range(q):
                        add(("down_pair", l, q), hidden_done(q) and hidden_done(l))
        plan.append(tasks)

    head, tail = plan[-1][:-G], plan[-1][-G:]
    corrections = [("correction", t, j) for t in (1, 0) for j in _longest_first(t)]
    mixed = [task for pair in zip(corrections, tail) for task in pair]
    assert head[-1][0] == "down_pair"
    plan[-1] = head + [("wait_b",) + head[-1][1:]] + mixed + corrections[G:]
    return plan


POS, USED = _operand_layout()
PLAN = _startup_plan()


def _dot_nt(a, b):
    return lax.dot_general(a, b, (((1,), (1,)), ((), ())), preferred_element_type=F32)


def _lin(a, b, sign, n):
    rows_a, rows_b = min(a.shape[0], n), min(b.shape[0], n)
    c = min(rows_a, rows_b)
    head = a[:c] + b[:c] if sign > 0 else a[:c] - b[:c]
    if c == n:
        return head
    if rows_a > rows_b:
        tail = a[c:n]
    else:
        tail = b[c:n] if sign > 0 else -b[c:n]
    return jnp.concatenate([head, tail], axis=0)


def _rows(g):
    return pl.ds(OFFSETS[g], SIZES[g])


def _cols(k):
    return pl.ds(k * T, T)


def _tile_key(g, k):
    return ("A", g, k) if g < G else ("B", g - G, k)


def _span(*keys):
    start, rows = POS[keys[0]]
    for key in keys[1:]:
        assert POS[key][0] == start + rows
        rows += POS[key][1]
    return pl.ds(start, rows)


def _low_lanes(shape):
    return lax.broadcasted_iota(jnp.int32, shape, 1) < HT


def _gate(t1, t2):
    low = _low_lanes(t1.shape)
    return jnp.where(low, t1, t2) * pltpu.roll(jnp.where(low, t2, t1), HT, 1)


class _GateUpPair:
    def __init__(self, x_ref, h_ref, h_tile, weight):
        self.x_ref, self.h_ref, self.h_tile, self.weight = x_ref, h_ref, h_tile, weight
        self.widened, self.acc, self.missing = {}, {}, {}
        for k in range(G):
            self.missing["a1", k] = self.missing["c2", k] = 2 * G
            self.missing["a2", k] = self.missing["c1", k] = G

    def _w(self, half, k):
        if (half, k) not in self.widened:
            self.widened[half, k] = self.weight(half, k).astype(F32)
        return self.widened[half, k]

    def _x(self, *keys):
        return self.x_ref[_span(*keys), :]

    def _give(self, v, *targets):
        for name, k, sign in targets:
            is_a = name[0] == "a"
            n = MA[k] if is_a else MB[k]
            if (name, k) in self.acc:
                self.acc[name, k] = _lin(self.acc[name, k], v, sign, n)
            else:
                first = v[:n] if sign > 0 else -v[:n]
                if first.shape[0] < n:
                    pad = jnp.zeros((n - first.shape[0], T), F32)
                    first = jnp.concatenate([first, pad], axis=0)
                self.acc[name, k] = first
            self.missing[name, k] -= 1
            n1, n2 = name[0] + "1", name[0] + "2"
            if self.missing[n1, k] == 0 and self.missing[n2, k] == 0:
                self.h_ref[self.h_tile, _rows(k if is_a else G + k), :] = _gate(
                    self.acc[n1, k], self.acc[n2, k])

    def m1(self, k, l, lhs):
        rhs = (self._w(0, l) + self._w(1, k)).astype(BF16)
        self._give(_dot_nt(lhs, rhs), ("a1", k, 1), ("c2", l, 1))

    def m2(self, l, lhs):
        self._give(_dot_nt(lhs, self._w(0, l).astype(BF16)), ("c1", l, 1), ("c2", l, 1))

    def m5(self, k, lhs):
        self._give(_dot_nt(lhs, self._w(1, k).astype(BF16)), ("a1", k, 1), ("a2", k, 1))

    def _w_diff(self, k):
        return (self._w(0, k) - self._w(1, k)).astype(BF16)

    def m3(self, k, lhs):
        self._give(_dot_nt(lhs, self._w_diff(k)), ("a1", k, 1))

    def m4(self, l, lhs):
        self._give(_dot_nt(lhs, self._w_diff(l)), ("c2", l, -1))

    def m3_m4(self, k, lhs):
        v = _dot_nt(lhs, self._w_diff(k))
        self._give(v[:MA[k]], ("a1", k, 1))
        self._give(v[MA[k]:], ("c2", k, -1))

    def m6(self, k, l):
        rhs = (self._w(0, k) + self._w(0, l)).astype(BF16)
        self._give(_dot_nt(self._x(("B", l, k)), rhs), ("c1", l, 1), ("a1", k, -1))

    def m7(self, k, l):
        rhs = (self._w(1, k) + self._w(1, l)).astype(BF16)
        self._give(_dot_nt(self._x(("A", k, l)), rhs), ("a2", k, 1), ("c2", l, -1))

    def m6_both(self, k, l):
        rhs = (self._w(0, k) + self._w(0, l)).astype(BF16)
        v = _dot_nt(self._x(("B", l, k), ("B", k, l)), rhs)
        self._give(v[:MB[l]], ("c1", l, 1), ("a1", k, -1))
        self._give(v[MB[l]:], ("c1", k, 1), ("a1", l, -1))

    def m7_both(self, k, l):
        rhs = (self._w(1, k) + self._w(1, l)).astype(BF16)
        v = _dot_nt(self._x(("A", k, l), ("A", l, k)), rhs)
        self._give(v[:MA[k]], ("a2", k, 1), ("c2", l, -1))
        self._give(v[MA[k]:], ("a2", l, 1), ("c2", k, -1))


class _DownPairs:
    def __init__(self, h_ref, js, weight, emit):
        self.h_ref, self.js, self.weight, self.emit = h_ref, js, weight, emit
        self.m2, self.m3, self.m4, self.m5 = {}, {}, {}, {}

    def _product(self, lhs, rhs):
        out = None
        for j in self.js:
            d = jnp.dot(lhs(j).astype(BF16), rhs(j).astype(BF16), preferred_element_type=F32)
            out = d if out is None else out + d
        return out

    def _h(self, half, g):
        return lambda j: self.h_ref[2 * j + half, _rows(g), :]

    def _w(self, half, k):
        return lambda j: self.weight(half, k, j)

    @staticmethod
    def _h_lin(f, g, sign, n):
        return lambda j: _lin(f(j), g(j), sign, n)

    @staticmethod
    def _w_lin(f, g, sign):
        return lambda j: _lin(f(j).astype(F32), g(j).astype(F32), sign, T)

    @staticmethod
    def _stack(f, g):
        return lambda j: jnp.concatenate([f(j), g(j)], axis=0)

    def diag(self, k):
        h, w = self._h, self._w
        self.m5[k] = self._product(self._h_lin(h(0, k), h(1, k), 1, MA[k]), w(1, k))
        self.m2[k] = self._product(self._h_lin(h(0, G + k), h(1, G + k), 1, MB[k]), w(0, k))
        m34 = self._product(self._stack(h(0, k), h(1, G + k)), self._w_lin(w(0, k), w(1, k), -1))
        self.m3[k], self.m4[k] = m34[:MA[k]], m34[MA[k]:]
        self.emit(k, k, self.m3[k] + self.m5[k])
        self.emit(G + k, k, self.m2[k] - self.m4[k])

    def pair(self, k, l):
        for q in (k, l):
            if q not in self.m2:
                self.diag(q)
        h, w = self._h, self._w
        m6 = self._product(
            self._stack(self._h_lin(h(0, G + l), h(0, k), -1, MB[l]),
                        self._h_lin(h(0, G + k), h(0, l), -1, MB[k])),
            self._w_lin(w(0, k), w(0, l), 1))
        m7 = self._product(
            self._stack(self._h_lin(h(1, k), h(1, G + l), -1, MA[k]),
                        self._h_lin(h(1, l), h(1, G + k), -1, MA[l])),
            self._w_lin(w(1, k), w(1, l), 1))
        for p, q, s6, s7 in ((k, l, slice(0, MB[l]), slice(0, MA[k])),
                             (l, k, slice(MB[l], None), slice(MA[k], None))):
            m1 = self._product(self._h_lin(h(0, p), h(1, G + q), 1, max(MA[p], MB[q])),
                               self._w_lin(w(0, q), w(1, p), 1))
            self.emit(p, q, _lin(m1, self.m4[q], -1, MA[p]) + (m7[s7] - self.m5[p]))
            self.emit(G + q, p, _lin(m1, self.m3[p], 1, MB[q]) + (m6[s6] - self.m2[q]))


def _kernel(x_hbm, wg_hbm, wu_hbm, wd_hbm, out_hbm,
            x_v,
            xsum_v,
            xf_v,
            w_v,
            ws_v,
            wd_v,
            wds_v,
            r_v,
            part_v,
            h_v,
            out_v,
            sem):
    copy = pltpu.make_async_copy
    n_stages = len(ARRIVALS)

    def gate_up_copies(c0, n, dst, d0, s):
        return [copy(w.at[pl.ds(c0, n)], dst.at[pl.ds(d0, n), pl.ds(r0, HT)], sem.at[s])
                for w, r0 in ((wg_hbm, 0), (wu_hbm, HT))]

    stage_copies = []
    for s, items in enumerate(ARRIVALS):
        group = []
        for item in items:
            if item == "wd":
                group += [copy(wd_hbm.at[pl.ds(24 * HT, 3 * HT), _cols(k)],
                               wds_v.at[k, pl.ds(0, 3 * HT)], sem.at[s]) for k in range(G)]
            elif isinstance(item, str):
                slot = {"w1": 0, "w2": 1, "w0": 2}[item]
                group += gate_up_copies(24 + slot, 1, ws_v, slot, s)
            else:
                group += [copy(x_hbm.at[_rows(item), _cols(k)],
                               x_v.at[_span(_tile_key(item, k))], sem.at[s]) for k in range(G)]
        stage_copies.append(group)
    b_copies = gate_up_copies(0, 10, w_v, 0, n_stages)
    v_copies = gate_up_copies(10, 14, w_v, 10, n_stages + 1)
    wd_copies = [copy(wd_hbm.at[pl.ds(0, 24 * HT), _cols(k)], wd_v.at[k], sem.at[n_stages + 2])
                 for k in range(G)]
    for c in sum(stage_copies, []) + b_copies + v_copies + wd_copies:
        c.start()
    for k in range(G):
        wds_v[k, pl.ds(3 * HT, HT), :] = jnp.zeros((HT, T), BF16)

    def x_f32(key):
        return x_v[_span(key), :].astype(F32)

    def x_operand(g, k, keep_f32):
        if not keep_f32:
            return x_v[_span(_tile_key(g, k)), :]
        wide = x_f32(_tile_key(g, k))
        xf_v[k, _rows(g), :] = wide
        return wide.astype(BF16)

    def keep_sum(key, v):
        xsum_v[_span(key), :] = v
        return v.astype(BF16)

    def row_sum(g):
        tiles = [x_f32(_tile_key(g, k)) for k in range(G)]
        v = tiles[g % G]
        for l in _others(g % G):
            v = v - tiles[l]
        return v

    def column_sum(kind, other, k):
        v = x_f32((kind, k, k))
        for l in _others(k):
            v = _lin(v, x_f32((other, l, k)), 1, v.shape[0])
        return v

    def plain(g):
        t = None
        for k in range(G):
            d = _dot_nt(x_operand(g, k, keep_f32=g < G), ws_v[2, :, _cols(k)])
            t = d if t is None else t + d
        h_v[13, _rows(g), :] = jnp.where(_low_lanes(t.shape), t * pltpu.roll(t, HT, 1), 0.0)

    def b_tile(t, j, k):
        return w_v[2 * k + t, :, _cols(j)]

    r_columns = {}

    def correction(t, j):
        g = G * t + j
        r = [_dot_nt(x_operand(g, k, keep_f32=g >= G), b_tile(t, j, k)) for k in range(G)]
        r_v[1, t, j, pl.ds(0, SIZES[g]), :] = sum(r[1:], r[0])
        for k in range(G):
            n, v = r_columns.get((t, k), (0, None))
            v = r[k] if v is None else _lin(v, r[k], 1, MAX_ROWS)
            r_columns[t, k] = (n + 1, v)
            if n + 1 == G:
                r_v[0, t, k] = v

    def wait_b(g, k):
        w_v[24, pl.ds(0, 16), pl.ds(0, T)] = part_v[k, pl.ds(OFFSETS[g], 16), :].astype(BF16)
        for c in b_copies:
            c.wait()

    def park(g, k, v):
        part_v[k, _rows(g), :] = v

    last_pair = _GateUpPair(x_v, h_v, 12, lambda half, k: ws_v[half, :, _cols(k)])
    last_down = _DownPairs(h_v, [6], lambda half, k, j: wds_v[k, pl.ds(half * T, T), :], park)
    actions = {
        "plain": plain,
        "1": lambda k, l: last_pair.m1(k, l, keep_sum(("1", k, l), _lin(
            x_f32(("A", k, l)), x_f32(("B", l, k)), 1, POS["1", k, l][1]))),
        "2": lambda l: last_pair.m2(l, keep_sum(("2", l), row_sum(G + l))),
        "3": lambda k: last_pair.m3(k, keep_sum(("3", k), column_sum("A", "B", k))),
        "4": lambda l: last_pair.m4(l, keep_sum(("4", l), column_sum("B", "A", l))),
        "5": lambda k: last_pair.m5(k, keep_sum(("5", k), row_sum(k))),
        "6": last_pair.m6,
        "7": last_pair.m7,
        "down_diag": last_down.diag,
        "down_pair": last_down.pair,
        "correction": correction,
        "wait_b": wait_b,
    }
    for group, tasks in zip(stage_copies, PLAN):
        for c in group:
            c.wait()
        for name, *args in tasks:
            actions[name](*args)

    for c in v_copies:
        c.wait()

    def gate_up_step(it, carry):
        def pick(c0, c1, k):
            return jnp.where(it == 0, w_v[c0, :, _cols(k)], w_v[c1, :, _cols(k)])

        def u_tile(t, j, k):
            return xf_v[k, _rows(G * t + j), :]

        @functools.cache
        def u_sum(t, k):
            v = None
            for j in _longest_first(t):
                v = u_tile(t, j, k) if v is None else _lin(v, u_tile(t, j, k), 1, MAX_ROWS)
            return v

        @functools.cache
        def b_sum(t, j):
            return sum((b_tile(t, j, k).astype(F32) for k in range(1, G)),
                       b_tile(t, j, 0).astype(F32))

        def x_sum(*keys):
            return xsum_v[_span(*keys), :].astype(BF16)

        pair = _GateUpPair(x_v, h_v, 10 + it, lambda half, k: pick(20 + half, 22 + half, k))
        for k in range(G):
            for l in range(k + 1, G):
                pair.m6_both(k, l)
                pair.m7_both(k, l)
                for p, q in ((k, l), (l, k)):
                    pair.m1(p, q, x_sum(("1", p, q)))
            pair.m5(k, x_sum(("5", k)))
            pair.m2(k, x_sum(("2", k)))
            pair.m3_m4(k, x_sum(("3", k), ("4", k)))

        def aggregate(i, pending):
            n = MA[i]
            a = [jnp.where(it == 0, xf_v[j, pl.ds(OFFSETS[i], n), :],
                           xf_v[j, pl.ds(S // 2 + OFFSETS[i], n), :]) for j in range(G)]
            v = [w.astype(F32) for w in [pick(10 + 2 * i, 11 + 2 * i, k) for k in range(G)]]
            a_sum, v_sum = sum(a[1:], a[0]), sum(v[1:], v[0])
            p = {}
            for j in range(G):
                for t in range(2):
                    nj = SIZES[G * t + j]
                    for k in range(G):
                        p[t, j, k] = _dot_nt(
                            _lin(a[j], u_tile(t, j, k), 1, max(n, nj)).astype(BF16),
                            (b_tile(t, j, k).astype(F32) + v[k]).astype(BF16))
                    q = _dot_nt(a[j][:min(n, nj)].astype(BF16), (b_sum(t, j) + v_sum).astype(BF16))
                    val = p[t, j, 0][:nj]
                    for k in range(1, G):
                        val = val + p[t, j, k][:nj]
                    val = _lin(val - r_v[1, t, j, pl.ds(0, nj), :], q, -1, nj)
                    half = lax.broadcasted_iota(jnp.int32, val.shape, 1) // HT
                    pltpu.store(h_v.at[G + i, _rows(G * t + j), :],
                                val * pltpu.roll(val, HT, 1), mask=half == it)
                if pending:
                    pending.pop(0)()

            def finish(k):
                vals = []
                for t in range(2):
                    s = _dot_nt((a_sum + u_sum(t, k)[:n]).astype(BF16), v[k].astype(BF16))
                    val = p[t, 0, k][:n]
                    for j in range(1, G):
                        val = val + p[t, j, k][:n]
                    vals.append(val - r_v[0, t, k, pl.ds(0, n), :] - s)
                rows = pl.ds(pl.multiple_of(it * (S // 2) + OFFSETS[i], 16), n)
                h_v[k, rows, :] = _gate(*vals)

            return [functools.partial(finish, k) for k in range(G)]

        pending = []
        for i in range(G):
            pending = aggregate(i, pending)
        for finish in pending:
            finish()
        return carry

    lax.fori_loop(0, 2, gate_up_step, None)

    for c in wd_copies:
        c.wait()
    out_copies = []

    def emit(g, k, v):
        out_v[k, _rows(g), :] = (v + part_v[k, _rows(g), :]).astype(BF16)
        c = copy(out_v.at[k, _rows(g)], out_hbm.at[_rows(g), _cols(k)], sem.at[n_stages + 3])
        c.start()
        out_copies.append(c)

    down = _DownPairs(h_v, range(6),
                      lambda half, k, j: wd_v[k, pl.ds((2 * j + half) * T, T), :], emit)
    for k, l in PAIRS:
        down.pair(k, l)
    for c in out_copies:
        c.wait()


@jax.jit
def pallas_standalone__glu_gated_bilinear__prompt_kernel(
    x: jax.Array,
    w_gate: jax.Array,
    w_up: jax.Array,
    w_down: jax.Array,
):
    assert x.shape == (1, S, D) and w_gate.shape == w_up.shape == (D, F)
    assert w_down.shape == (F, D)
    hbm = pl.BlockSpec(memory_space=pltpu.HBM)
    out = pl.pallas_call(
        _kernel,
        in_specs=[hbm] * 4,
        out_specs=hbm,
        out_shape=jax.ShapeDtypeStruct((S, D), BF16),
        scratch_shapes=[
            pltpu.VMEM((USED["tile"], T), BF16),
            pltpu.VMEM((USED["sum"], T), F32),
            pltpu.VMEM((G, S, T), F32),
            pltpu.VMEM((25, T, D), BF16),
            pltpu.VMEM((3, T, D), BF16),
            pltpu.VMEM((G, 24 * HT, T), BF16),
            pltpu.VMEM((G, 2 * T, T), BF16),
            pltpu.VMEM((2, 2, G, MAX_ROWS, T), F32),
            pltpu.VMEM((G, S, T), F32),
            pltpu.VMEM((14, S, T), F32),
            pltpu.VMEM((G, S, T), BF16),
            pltpu.SemaphoreType.DMA((len(ARRIVALS) + 4,)),
        ],
        compiler_params=pltpu.CompilerParams(
            vmem_limit_bytes=110 * 1024 * 1024,
            disable_bounds_checks=True,
            disable_semaphore_checks=True,
            flags={"XLA_TPU_RESCHEDULE_DMA_DONES": True},
        ),
    )(
        x.reshape(S, D),
        w_gate.T.reshape(F // HT, HT, D),
        w_up.T.reshape(F // HT, HT, D),
        w_down,
    )
    return out.reshape(1, S, D)
```

```python
import functools
import itertools

import jax
import jax.numpy as jnp
from jax import lax
import jax.experimental.pallas as pl
import jax.experimental.pallas.tpu as pltpu

S, D, F = 2048, 640, 1728
T = 128
HT = T // 2
G = D // T

SIZES = (208, 208, 208, 208, 192, 192, 208, 208, 208, 208)
OFFSETS = (0, 208, 416, 624, 832, 1856, 1024, 1232, 1440, 1648)
MA, MB = SIZES[:G], SIZES[G:]
MAX_ROWS = max(SIZES)
PAIRS = tuple(itertools.combinations(range(G), 2))

ARRIVALS = (("w0", 0), ("w2",), (1,), (2,), (3,), (4,), (5,), ("w1",),
            (6,), (7,), (8,), (9, "wd"))

F32, BF16 = jnp.float32, jnp.bfloat16


def _others(k):
    return [l for l in range(G) if l != k]


def _longest_first(half):
    return sorted(range(G), key=lambda j: -SIZES[G * half + j])


def _operand_layout():
    pos, used = {}, {"tile": 0, "sum": 0}

    def put(key, rows):
        kind = "tile" if key[0] in "AB" else "sum"
        pos[key] = (used[kind], rows)
        used[kind] += rows

    for k in range(G):
        put(("3", k), MA[k])
        put(("4", k), MB[k])
        put(("5", k), MA[k])
        put(("2", k), MB[k])
        put(("A", k, k), MA[k])
        put(("B", k, k), MB[k])
    for k, l in PAIRS:
        put(("B", l, k), MB[l])
        put(("B", k, l), MB[k])
        put(("A", k, l), MA[k])
        put(("A", l, k), MA[l])
    return pos, used


def _startup_plan():
    plan, done, have = [], set(), set()
    for items in ARRIVALS:
        have.update(items)
        tasks = []
        has_a = lambda k: k in have
        has_b = lambda k: G + k in have
        w1, w2 = "w1" in have, "w2" in have

        def add(task, ready):
            if ready and task not in done:
                done.add(task)
                tasks.append(task)

        def hidden_done(q):
            need = [("plain", q), ("plain", G + q)] + [(m, q) for m in "2345"]
            for l in _others(q):
                need += [(m, p, r) for m in "167" for p, r in ((q, l), (l, q))]
            return all(t in done for t in need)

        for k in range(G):
            for l in range(k + 1, G):
                for p, q in ((k, l), (l, k)):
                    add(("7", p, q), w2 and has_a(p))
                for p, q in ((k, l), (l, k)):
                    add(("6", p, q), w1 and has_b(q))
                for p, q in ((k, l), (l, k)):
                    add(("1", p, q), w1 and w2 and has_a(p) and has_b(q))
            add(("5", k), w2 and has_a(k))
            add(("2", k), w1 and has_b(k))
            add(("4", k), w1 and w2 and has_b(k) and all(map(has_a, _others(k))))
            add(("3", k), w1 and w2 and has_a(k) and all(map(has_b, _others(k))))
            if tasks or k == G - 1:
                for g in range(2 * G):
                    add(("plain", g), g in have)
            if "wd" in have:
                for q in range(k if k < G - 1 else G):
                    add(("down_diag", q), hidden_done(q))
                    for l in range(q):
                        add(("down_pair", l, q), hidden_done(q) and hidden_done(l))
        plan.append(tasks)

    head, tail = plan[-1][:-G], plan[-1][-G:]
    corrections = [("correction", t, j) for t in (1, 0) for j in _longest_first(t)]
    mixed = [task for pair in zip(corrections, tail) for task in pair]
    assert head[-1][0] == "down_pair"
    plan[-1] = head + [("wait_b",) + head[-1][1:]] + mixed + corrections[G:]
    return plan


POS, USED = _operand_layout()
PLAN = _startup_plan()


def _dot_nt(a, b):
    return lax.dot_general(a, b, (((1,), (1,)), ((), ())), preferred_element_type=F32)


def _lin(a, b, sign, n):
    rows_a, rows_b = min(a.shape[0], n), min(b.shape[0], n)
    c = min(rows_a, rows_b)
    head = a[:c] + b[:c] if sign > 0 else a[:c] - b[:c]
    if c == n:
        return head
    if rows_a > rows_b:
        tail = a[c:n]
    else:
        tail = b[c:n] if sign > 0 else -b[c:n]
    return jnp.concatenate([head, tail], axis=0)


def _rows(g):
    return pl.ds(OFFSETS[g], SIZES[g])


def _cols(k):
    return pl.ds(k * T, T)


def _tile_key(g, k):
    return ("A", g, k) if g < G else ("B", g - G, k)


def _span(*keys):
    start, rows = POS[keys[0]]
    for key in keys[1:]:
        assert POS[key][0] == start + rows
        rows += POS[key][1]
    return pl.ds(start, rows)


def _low_lanes(shape):
    return lax.broadcasted_iota(jnp.int32, shape, 1) < HT


def _gate(t1, t2):
    low = _low_lanes(t1.shape)
    return jnp.where(low, t1, t2) * pltpu.roll(jnp.where(low, t2, t1), HT, 1)


class _GateUpPair:
    def __init__(self, x_ref, h_ref, h_tile, weight):
        self.x_ref, self.h_ref, self.h_tile, self.weight = x_ref, h_ref, h_tile, weight
        self.widened, self.acc, self.missing = {}, {}, {}
        for k in range(G):
            self.missing["a1", k] = self.missing["c2", k] = 2 * G
            self.missing["a2", k] = self.missing["c1", k] = G

    def _w(self, half, k):
        if (half, k) not in self.widened:
            self.widened[half, k] = self.weight(half, k).astype(F32)
        return self.widened[half, k]

    def _x(self, *keys):
        return self.x_ref[_span(*keys), :]

    def _give(self, v, *targets):
        for name, k, sign in targets:
            is_a = name[0] == "a"
            n = MA[k] if is_a else MB[k]
            if (name, k) in self.acc:
                self.acc[name, k] = _lin(self.acc[name, k], v, sign, n)
            else:
                first = v[:n] if sign > 0 else -v[:n]
                if first.shape[0] < n:
                    pad = jnp.zeros((n - first.shape[0], T), F32)
                    first = jnp.concatenate([first, pad], axis=0)
                self.acc[name, k] = first
            self.missing[name, k] -= 1
            n1, n2 = name[0] + "1", name[0] + "2"
            if self.missing[n1, k] == 0 and self.missing[n2, k] == 0:
                self.h_ref[self.h_tile, _rows(k if is_a else G + k), :] = _gate(
                    self.acc[n1, k], self.acc[n2, k])

    def m1(self, k, l, xa, xb):
        lhs = _lin(xa, xb, -1, max(MA[k], MB[l])).astype(BF16)
        rhs = (self._w(0, l) + self._w(1, k)).astype(BF16)
        self._give(_dot_nt(lhs, rhs), ("a1", k, 1), ("c2", l, -1))

    def m2(self, l, lhs):
        self._give(_dot_nt(lhs, self._w(0, l).astype(BF16)), ("c1", l, 1), ("c2", l, 1))

    def m5(self, k, lhs):
        self._give(_dot_nt(lhs, self._w(1, k).astype(BF16)), ("a1", k, 1), ("a2", k, 1))

    def _w_diff(self, k):
        return (self._w(0, k) - self._w(1, k)).astype(BF16)

    def m3(self, k, lhs):
        self._give(_dot_nt(lhs, self._w_diff(k)), ("a1", k, 1))

    def m4(self, l, lhs):
        self._give(_dot_nt(lhs, self._w_diff(l)), ("c2", l, -1))

    def m3_m4(self, k, lhs):
        v = _dot_nt(lhs, self._w_diff(k))
        self._give(v[:MA[k]], ("a1", k, 1))
        self._give(v[MA[k]:], ("c2", k, -1))

    def m6(self, k, l):
        rhs = (self._w(0, k) + self._w(0, l)).astype(BF16)
        self._give(_dot_nt(self._x(("B", l, k)), rhs), ("c1", l, 1), ("a1", k, 1))

    def m7(self, k, l):
        rhs = (self._w(1, k) + self._w(1, l)).astype(BF16)
        self._give(_dot_nt(self._x(("A", k, l)), rhs), ("a2", k, 1), ("c2", l, 1))

    def m6_both(self, k, l):
        rhs = (self._w(0, k) + self._w(0, l)).astype(BF16)
        v = _dot_nt(self._x(("B", l, k), ("B", k, l)), rhs)
        self._give(v[:MB[l]], ("c1", l, 1), ("a1", k, 1))
        self._give(v[MB[l]:], ("c1", k, 1), ("a1", l, 1))

    def m7_both(self, k, l):
        rhs = (self._w(1, k) + self._w(1, l)).astype(BF16)
        v = _dot_nt(self._x(("A", k, l), ("A", l, k)), rhs)
        self._give(v[:MA[k]], ("a2", k, 1), ("c2", l, 1))
        self._give(v[MA[k]:], ("a2", l, 1), ("c2", k, 1))


class _DownPairs:
    def __init__(self, h_ref, js, weight, emit):
        self.h_ref, self.js, self.weight, self.emit = h_ref, js, weight, emit
        self.m2, self.m3, self.m4, self.m5 = {}, {}, {}, {}

    def _product(self, lhs, rhs):
        out = None
        for j in self.js:
            d = jnp.dot(lhs(j).astype(BF16), rhs(j).astype(BF16), preferred_element_type=F32)
            out = d if out is None else out + d
        return out

    def _h(self, half, g):
        return lambda j: self.h_ref[2 * j + half, _rows(g), :]

    def _w(self, half, k):
        return lambda j: self.weight(half, k, j)

    @staticmethod
    def _h_lin(f, g, sign, n):
        return lambda j: _lin(f(j), g(j), sign, n)

    @staticmethod
    def _w_lin(f, g, sign):
        return lambda j: _lin(f(j).astype(F32), g(j).astype(F32), sign, T)

    @staticmethod
    def _stack(f, g):
        return lambda j: jnp.concatenate([f(j), g(j)], axis=0)

    def diag(self, k):
        h, w = self._h, self._w
        self.m5[k] = self._product(self._h_lin(h(0, k), h(1, k), 1, MA[k]), w(1, k))
        self.m2[k] = self._product(self._h_lin(h(0, G + k), h(1, G + k), 1, MB[k]), w(0, k))
        m34 = self._product(self._stack(h(0, k), h(1, G + k)), self._w_lin(w(0, k), w(1, k), -1))
        self.m3[k], self.m4[k] = m34[:MA[k]], m34[MA[k]:]
        self.emit(k, k, self.m3[k] + self.m5[k])
        self.emit(G + k, k, self.m2[k] - self.m4[k])

    def pair(self, k, l):
        for q in (k, l):
            if q not in self.m2:
                self.diag(q)
        h, w = self._h, self._w
        m6 = self._product(
            self._stack(self._h_lin(h(0, G + l), h(0, k), -1, MB[l]),
                        self._h_lin(h(0, G + k), h(0, l), -1, MB[k])),
            self._w_lin(w(0, k), w(0, l), 1))
        m7 = self._product(
            self._stack(self._h_lin(h(1, k), h(1, G + l), -1, MA[k]),
                        self._h_lin(h(1, l), h(1, G + k), -1, MA[l])),
            self._w_lin(w(1, k), w(1, l), 1))
        for p, q, s6, s7 in ((k, l, slice(0, MB[l]), slice(0, MA[k])),
                             (l, k, slice(MB[l], None), slice(MA[k], None))):
            m1 = self._product(self._h_lin(h(0, p), h(1, G + q), 1, max(MA[p], MB[q])),
                               self._w_lin(w(0, q), w(1, p), 1))
            self.emit(p, q, _lin(m1, self.m4[q], -1, MA[p]) + (m7[s7] - self.m5[p]))
            self.emit(G + q, p, _lin(m1, self.m3[p], 1, MB[q]) + (m6[s6] - self.m2[q]))


def _kernel(x_hbm, wg_hbm, wu_hbm, wd_hbm, out_hbm,
            x_v,
            xsum_v,
            xf_v,
            w_v,
            ws_v,
            wd_v,
            wds_v,
            r_v,
            part_v,
            h_v,
            out_v,
            sem):
    copy = pltpu.make_async_copy
    n_stages = len(ARRIVALS)

    def gate_up_copies(c0, n, dst, d0, s):
        return [copy(w.at[pl.ds(c0, n)], dst.at[pl.ds(d0, n), pl.ds(r0, HT)], sem.at[s])
                for w, r0 in ((wg_hbm, 0), (wu_hbm, HT))]

    stage_copies = []
    for s, items in enumerate(ARRIVALS):
        group = []
        for item in items:
            if item == "wd":
                group += [copy(wd_hbm.at[pl.ds(24 * HT, 3 * HT), _cols(k)],
                               wds_v.at[k, pl.ds(0, 3 * HT)], sem.at[s]) for k in range(G)]
            elif isinstance(item, str):
                slot = {"w1": 0, "w2": 1, "w0": 2}[item]
                group += gate_up_copies(24 + slot, 1, ws_v, slot, s)
            else:
                group += [copy(x_hbm.at[_rows(item), _cols(k)],
                               x_v.at[_span(_tile_key(item, k))], sem.at[s]) for k in range(G)]
        stage_copies.append(group)
    b_copies = gate_up_copies(0, 10, w_v, 0, n_stages)
    v_copies = gate_up_copies(10, 14, w_v, 10, n_stages + 1)
    wd_copies = [copy(wd_hbm.at[pl.ds(0, 24 * HT), _cols(k)], wd_v.at[k], sem.at[n_stages + 2])
                 for k in range(G)]
    for c in sum(stage_copies, []) + b_copies + v_copies + wd_copies:
        c.start()
    for k in range(G):
        wds_v[k, pl.ds(3 * HT, HT), :] = jnp.zeros((HT, T), BF16)

    def x_f32(key):
        return x_v[_span(key), :].astype(F32)

    def x_operand(g, k, keep_f32):
        if not keep_f32:
            return x_v[_span(_tile_key(g, k)), :]
        wide = x_f32(_tile_key(g, k))
        xf_v[k, _rows(g), :] = wide
        return wide.astype(BF16)

    def keep_sum(key, v):
        xsum_v[_span(key), :] = v
        return v.astype(BF16)

    def row_combo(g):
        tiles = [x_f32(_tile_key(g, k)) for k in range(G)]
        v = tiles[g % G]
        for l in _others(g % G):
            v = v - tiles[l]
        return v

    def column_combo(kind, other, k):
        v = x_f32((kind, k, k))
        for l in _others(k):
            v = _lin(v, x_f32((other, l, k)), -1, v.shape[0])
        return v

    def plain(g):
        t = None
        for k in range(G):
            d = _dot_nt(x_operand(g, k, keep_f32=g < G), ws_v[2, :, _cols(k)])
            t = d if t is None else t + d
        h_v[13, _rows(g), :] = jnp.where(_low_lanes(t.shape), t * pltpu.roll(t, HT, 1), 0.0)

    def b_tile(t, j, k):
        return w_v[2 * k + t, :, _cols(j)]

    r_columns = {}

    def correction(t, j):
        g = G * t + j
        r = [_dot_nt(x_operand(g, k, keep_f32=g >= G), b_tile(t, j, k)) for k in range(G)]
        r_v[1, t, j, pl.ds(0, SIZES[g]), :] = sum(r[1:], r[0])
        for k in range(G):
            n, v = r_columns.get((t, k), (0, None))
            v = r[k] if v is None else _lin(v, r[k], 1, MAX_ROWS)
            r_columns[t, k] = (n + 1, v)
            if n + 1 == G:
                r_v[0, t, k] = v

    def wait_b(g, k):
        w_v[24, pl.ds(0, 16), pl.ds(0, T)] = part_v[k, pl.ds(OFFSETS[g], 16), :].astype(BF16)
        for c in b_copies:
            c.wait()

    def park(g, k, v):
        part_v[k, _rows(g), :] = v

    last_pair = _GateUpPair(x_v, h_v, 12, lambda half, k: ws_v[half, :, _cols(k)])
    last_down = _DownPairs(h_v, [6], lambda half, k, j: wds_v[k, pl.ds(half * T, T), :], park)
    actions = {
        "plain": plain,
        "1": lambda k, l: last_pair.m1(k, l, x_f32(("A", k, l)), x_f32(("B", l, k))),
        "2": lambda l: last_pair.m2(l, keep_sum(("2", l), row_combo(G + l))),
        "3": lambda k: last_pair.m3(k, keep_sum(("3", k), column_combo("A", "B", k))),
        "4": lambda l: last_pair.m4(l, keep_sum(("4", l), column_combo("B", "A", l))),
        "5": lambda k: last_pair.m5(k, keep_sum(("5", k), row_combo(k))),
        "6": last_pair.m6,
        "7": last_pair.m7,
        "down_diag": last_down.diag,
        "down_pair": last_down.pair,
        "correction": correction,
        "wait_b": wait_b,
    }
    for group, tasks in zip(stage_copies, PLAN):
        for c in group:
            c.wait()
        for name, *args in tasks:
            actions[name](*args)

    for c in v_copies:
        c.wait()

    def gate_up_step(it, carry):
        def pick(c0, c1, k):
            return jnp.where(it == 0, w_v[c0, :, _cols(k)], w_v[c1, :, _cols(k)])

        def u_tile(t, j, k):
            return xf_v[k, _rows(G * t + j), :]

        @functools.cache
        def u_sum(t, k):
            v = None
            for j in _longest_first(t):
                v = u_tile(t, j, k) if v is None else _lin(v, u_tile(t, j, k), 1, MAX_ROWS)
            return v

        @functools.cache
        def b_sum(t, j):
            return sum((b_tile(t, j, k).astype(F32) for k in range(1, G)),
                       b_tile(t, j, 0).astype(F32))

        def x_sum(*keys):
            return xsum_v[_span(*keys), :].astype(BF16)

        pair = _GateUpPair(x_v, h_v, 10 + it, lambda half, k: pick(20 + half, 22 + half, k))
        for k in range(G):
            for l in range(k + 1, G):
                pair.m6_both(k, l)
                pair.m7_both(k, l)
                for p, q in ((k, l), (l, k)):
                    pair.m1(p, q, u_tile(0, p, q), u_tile(1, q, p))
            pair.m5(k, x_sum(("5", k)))
            pair.m2(k, x_sum(("2", k)))
            pair.m3_m4(k, x_sum(("3", k), ("4", k)))

        def aggregate(i, pending):
            n = MA[i]
            a = [jnp.where(it == 0, xf_v[j, pl.ds(OFFSETS[i], n), :],
                           xf_v[j, pl.ds(S // 2 + OFFSETS[i], n), :]) for j in range(G)]
            v = [w.astype(F32) for w in [pick(10 + 2 * i, 11 + 2 * i, k) for k in range(G)]]
            a_sum, v_sum = sum(a[1:], a[0]), sum(v[1:], v[0])
            p = {}
            for j in range(G):
                for t in range(2):
                    nj = SIZES[G * t + j]
                    for k in range(G):
                        p[t, j, k] = _dot_nt(
                            _lin(a[j], u_tile(t, j, k), -1, max(n, nj)).astype(BF16),
                            (b_tile(t, j, k).astype(F32) - v[k]).astype(BF16))
                    q = _dot_nt(a[j][:min(n, nj)].astype(BF16), (b_sum(t, j) - v_sum).astype(BF16))
                    val = p[t, j, 0][:nj]
                    for k in range(1, G):
                        val = val + p[t, j, k][:nj]
                    val = _lin(val + r_v[1, t, j, pl.ds(0, nj), :], q, -1, nj)
                    keep = _low_lanes(val.shape) & (it == 1)
                    rows = _rows(G * t + j)
                    h_v[G + i, rows, :] = jnp.where(
                        keep, h_v[G + i, rows, :], val * pltpu.roll(val, HT, 1))
                if pending:
                    pending.pop(0)()

            def finish(k):
                vals = []
                for t in range(2):
                    s = _dot_nt((a_sum - u_sum(t, k)[:n]).astype(BF16), v[k].astype(BF16))
                    val = p[t, 0, k][:n]
                    for j in range(1, G):
                        val = val + p[t, j, k][:n]
                    vals.append(val + r_v[0, t, k, pl.ds(0, n), :] + s)
                rows = pl.ds(pl.multiple_of(it * (S // 2) + OFFSETS[i], 16), n)
                h_v[k, rows, :] = _gate(*vals)

            return [functools.partial(finish, k) for k in range(G)]

        pending = []
        for i in range(G):
            pending = aggregate(i, pending)
        for finish in pending:
            finish()
        return carry

    lax.fori_loop(0, 2, gate_up_step, None)

    for c in wd_copies:
        c.wait()
    out_copies = []

    def emit(g, k, v):
        out_v[k, _rows(g), :] = (v + part_v[k, _rows(g), :]).astype(BF16)
        c = copy(out_v.at[k, _rows(g)], out_hbm.at[_rows(g), _cols(k)], sem.at[n_stages + 3])
        c.start()
        out_copies.append(c)

    down = _DownPairs(h_v, range(6),
                      lambda half, k, j: wd_v[k, pl.ds((2 * j + half) * T, T), :], emit)
    for k, l in PAIRS:
        down.pair(k, l)
    for c in out_copies:
        c.wait()


@jax.jit
def pallas_standalone__glu_gated_bilinear__prompt_kernel(
    x: jax.Array,
    w_gate: jax.Array,
    w_up: jax.Array,
    w_down: jax.Array,
):
    assert x.shape == (1, S, D) and w_gate.shape == w_up.shape == (D, F)
    assert w_down.shape == (F, D)
    hbm = pl.BlockSpec(memory_space=pltpu.HBM)
    out = pl.pallas_call(
        _kernel,
        in_specs=[hbm] * 4,
        out_specs=hbm,
        out_shape=jax.ShapeDtypeStruct((S, D), BF16),
        scratch_shapes=[
            pltpu.VMEM((USED["tile"], T), BF16),
            pltpu.VMEM((USED["sum"], T), F32),
            pltpu.VMEM((G, S, T), F32),
            pltpu.VMEM((25, T, D), BF16),
            pltpu.VMEM((3, T, D), BF16),
            pltpu.VMEM((G, 24 * HT, T), BF16),
            pltpu.VMEM((G, 2 * T, T), BF16),
            pltpu.VMEM((2, 2, G, MAX_ROWS, T), F32),
            pltpu.VMEM((G, S, T), F32),
            pltpu.VMEM((14, S, T), F32),
            pltpu.VMEM((G, S, T), BF16),
            pltpu.SemaphoreType.DMA((len(ARRIVALS) + 4,)),
        ],
        compiler_params=pltpu.CompilerParams(
            vmem_limit_bytes=110 * 1024 * 1024,
            disable_semaphore_checks=True,
            flags={"XLA_TPU_RESCHEDULE_DMA_DONES": True},
        ),
    )(
        x.reshape(S, D),
        w_gate.T.reshape(F // HT, HT, D),
        w_up.T.reshape(F // HT, HT, D),
        w_down,
    )
    return out.reshape(1, S, D)
```
